```python
import jax
import jax.numpy as jnp

def _softmax(x, axis=-1):
    return jax.nn.softmax(x, axis=axis)
def _gelu(x):
    return jax.nn.gelu(x, approximate=True)
def _silu(x):
    return jax.nn.silu(x)
def _sigmoid(x):
    return jax.nn.sigmoid(x)
def _layernorm(x, axis=-1, eps=1e-5):
    m = jnp.mean(x, axis=axis, keepdims=True)
    v = jnp.var(x, axis=axis, keepdims=True)
    return (x - m) / jnp.sqrt(v + eps)
def _scatter_add(tgt, idx, src, axis=0):
    return tgt.at[idx].add(src)
def _segment_sum(src, seg, n):
    return jax.ops.segment_sum(src, seg, n)
class _Rng:
    def __init__(self, key):
        self._k = key
    def _next(self):
        self._k, sub = jax.random.split(self._k)
        return sub
    def normal(self, shape):
        return jax.random.normal(self._next(), shape, dtype=jnp.bfloat16)
    def randint(self, lo, hi, shape):
        return jax.random.randint(self._next(), shape, lo, hi, dtype=jnp.int32)
    def uniform(self, shape, lo=0.0, hi=1.0):
        return jax.random.uniform(self._next(), shape, jnp.bfloat16, lo, hi)
    def permutation(self, n):
        return jax.random.permutation(self._next(), n)


kernel_name = 'standalone__cross_network_dcn__recsys'

def setup_inputs():
    _rng = _Rng(jax.random.key(int.from_bytes(__import__("os").urandom(4), "little")))
    _w = (lambda a: (lambda t: t.astype(jnp.bfloat16) if jnp.issubdtype(t.dtype, jnp.floating) else t)(jnp.asarray(a)))
    B, F, D, L = 16384, 100, 16, 6
    Din = min(F * D, 1024)
    return {
        "x0": _w((lambda *s: _rng.normal(s) * 0.05)(B, Din)),
        "ws": _w((lambda *s: _rng.normal(s) * 0.05)(L, Din, Din) * (Din ** -0.5)),
        "bs": _w((lambda *s: _rng.normal(s) * 0.05)(L, Din) * 0.01),
    }

def reference(x0, ws, bs):
    x = x0
    L = ws.shape[0]
    for l in range(L):
        proj = jnp.einsum('bd,de->be', x, ws[l]) + bs[l]
        x = x0 * proj + x
    return x
```

```python
import jax
import jax.numpy as jnp
import jax.experimental.pallas as pl
import jax.experimental.pallas.tpu as pltpu

TM = 512
SUB = 1

def _kernel(x0_ref, ws_ref, bs_ref, o_ref):
    L = ws_ref.shape[0]
    sm = TM // SUB
    x0s = [x0_ref[pl.ds(s * sm, sm), :].astype(jnp.float32) for s in range(SUB)]
    xs = list(x0s)
    for l in range(L):
        b = bs_ref[pl.ds(l, 1), :].astype(jnp.float32)
        for s in range(SUB):
            p = jnp.dot(xs[s].astype(jnp.bfloat16), ws_ref[l], preferred_element_type=jnp.float32)
            xs[s] = x0s[s] * (p + b) + xs[s]
    for s in range(SUB):
        o_ref[pl.ds(s * sm, sm), :] = xs[s].astype(o_ref.dtype)

@jax.jit
def pallas_standalone__cross_network_dcn__recsys_kernel(x0, ws, bs):
    B, D = x0.shape
    L = ws.shape[0]
    return pl.pallas_call(
        _kernel,
        grid=(B // TM,),
        in_specs=[
            pl.BlockSpec((TM, D), lambda i: (i, 0)),
            pl.BlockSpec((L, D, D), lambda i: (0, 0, 0), pipeline_mode=pl.Buffered(1)),
            pl.BlockSpec((L, D), lambda i: (0, 0)),
        ],
        out_specs=pl.BlockSpec((TM, D), lambda i: (i, 0)),
        out_shape=jax.ShapeDtypeStruct((B, D), x0.dtype),
        compiler_params=pltpu.CompilerParams(dimension_semantics=("arbitrary",), vmem_limit_bytes=100 * 1024 * 1024),
    )(x0, ws, bs)
```

```python
import functools

import jax
import jax.numpy as jnp
import jax.experimental.pallas as pl
import jax.experimental.pallas.tpu as pltpu

H2 = 64
NS = 3
VI = 2
VO = 2
FLAGS = {"XLA_TPU_FORCE_LP_LLO_SCHEDULER": True}
f32 = jnp.float32
bf16 = jnp.bfloat16
u32 = jnp.uint32
QUAD = ((0, 0), (0, 1), (1, 0), (1, 1))


class _Blocks:
    def __init__(self, v):
        self.v = list(v)

    def __add__(self, o):
        return _Blocks(a + b for a, b in zip(self.v, o.v))

    def __sub__(self, o):
        return _Blocks(a - b for a, b in zip(self.v, o.v))


def _rhs_sums(B11, B12, B21, B22):
    yield B11 + B22
    yield B11
    yield B12 - B22
    yield B21 - B11
    yield B22
    yield B11 + B12
    yield B21 + B22


def _strassen(A, mul, done, var):
    A11, A12, A21, A22 = A
    M2 = mul(1, A21 + A22)
    M4 = mul(3, A22)
    done(2, M2 + M4)
    M3 = mul(2, A11)
    M5 = mul(4, A11 + A12)
    done(1, M3 + M5)
    M1 = mul(0, A11 + A22)
    if var:
        done(3, ((M3 - M2) + M1) + mul(5, A21 - A11))
        done(0, ((M4 - M5) + M1) + mul(6, A12 - A22))
    else:
        done(3, (M3 - M2) + (M1 + mul(5, A21 - A11)))
        done(0, (M4 - M5) + (M1 + mul(6, A12 - A22)))


def _kernel(x0_ref, ws_hbm, bs_ref, o_ref, w_ref, wc_ref, bb_ref, x_ref, sems, *, head):
    L, D, _ = w_ref.shape
    d = D // 4

    def tile_blocks(s):
        return [[(pl.ds((4 * s + 2 * I + i) * H2, H2), pl.ds((2 * J + j) * d, d)) for i, j in QUAD]
                for I, J in QUAD]

    def cross_layer(l, X0, X):
        def outer_mul(p, A):
            def mul(p2, a):
                w = jnp.concatenate([wc_ref.bitcast(u32)[l, 7 * p + p2, c] for c in range(d // 128)], axis=1)
                m = jnp.dot(a.astype(bf16), pltpu.bitcast(w, bf16), preferred_element_type=f32)
                if p in (2, 3) and p2 in (2, 3):
                    m = m + jnp.tile(bb_ref[l, :, pl.ds((2 * (3 - p) + 3 - p2) * d, d)], (H2 // 8, 1))
                return m
            C = [None] * 4
            _strassen(A.v, mul, C.__setitem__, VI)
            return _Blocks(C)

        Xn = [None] * 4

        def cross(q, proj):
            Xn[q] = _Blocks(x0 * c + x for x0, c, x in zip(X0[q].v, proj.v, X[q].v))

        _strassen(X, outer_mul, cross, VO)
        return Xn

    def load(ref, s):
        return [_Blocks(ref[b].astype(f32) for b in bq) for bq in tile_blocks(s)]

    def store(ref, s, X):
        for bq, Xq in zip(tile_blocks(s), X):
            for b, v in zip(bq, Xq.v):
                ref[b] = v.astype(ref.dtype)

    @pl.when(pl.program_id(0) == 0)
    def _first_step():
        copy = lambda l: pltpu.make_async_copy(ws_hbm.at[l], w_ref.at[l], sems.at[l])
        for l in range(L):
            copy(l).start()
        for l in range(L):
            bb_ref[l] = jnp.broadcast_to(bs_ref[l:l + 1, :].astype(f32), (8, D))
        x_ref[...] = x0_ref[:head, :].astype(f32)

        @pl.loop(0, L)
        def _(l):
            copy(l).wait()
            for c in range(d // 128):
                @pl.loop(0, d // 16)
                def _(t):
                    r = pl.multiple_of(t * 16, 16)
                    W = [_Blocks(w_ref[l, pl.ds((2 * I + i) * d + r, 16), pl.ds((2 * J + j) * d + c * 128, 128)].astype(f32)
                                 for i, j in QUAD) for I, J in QUAD]
                    for p, Wp in enumerate(_rhs_sums(*W)):
                        for p2, w in enumerate(_rhs_sums(*Wp.v)):
                            wc_ref[l, 7 * p + p2, c, pl.ds(r, 16), :] = w.astype(bf16)
            for s in range(head // (4 * H2)):
                store(x_ref, s, cross_layer(l, load(x0_ref, s), load(x_ref, s)))

        o_ref[:head, :] = x_ref[...].astype(o_ref.dtype)

    @pl.when(pl.program_id(0) > 0)
    def _steady_step():
        for s in range(NS):
            X0 = X = load(x0_ref, s)
            for l in range(L):
                X = cross_layer(l, X0, X)
            store(o_ref, s, X)


@jax.jit
def pallas_standalone__cross_network_dcn__recsys_kernel(x0, ws, bs):
    B, D = x0.shape
    L = ws.shape[0]
    d = D // 4
    TM = 4 * H2 * NS
    steps = pl.cdiv(B, TM)
    head = B - (steps - 1) * TM
    rows = lambda i: (jnp.where(i == 0, steps - 1, i - 1), 0)
    return pl.pallas_call(
        functools.partial(_kernel, head=head),
        grid=(steps,),
        in_specs=[
            pl.BlockSpec((TM, D), rows),
            pl.BlockSpec(memory_space=pl.ANY),
            pl.BlockSpec((L, D), lambda i: (0, 0)),
        ],
        out_specs=pl.BlockSpec((TM, D), rows),
        out_shape=jax.ShapeDtypeStruct((B, D), x0.dtype),
        scratch_shapes=[
            pltpu.VMEM((L, D, D), ws.dtype),
            pltpu.VMEM((L, 49, d // 128, d, 128), bf16),
            pltpu.VMEM((L, 8, D), f32),
            pltpu.VMEM((head, D), f32),
            pltpu.SemaphoreType.DMA((L,)),
        ],
        compiler_params=pltpu.CompilerParams(
            dimension_semantics=("arbitrary",), vmem_limit_bytes=100 * 1024 * 1024, flags=FLAGS),
    )(x0, ws, bs)
```

```python
import functools

import jax
import jax.numpy as jnp
import jax.experimental.pallas as pl
import jax.experimental.pallas.tpu as pltpu

H2 = 64
NS = 3
AHEAD = 2
FLAGS = {"XLA_TPU_FORCE_LP_LLO_SCHEDULER": True}
f32 = jnp.float32
bf16 = jnp.bfloat16
u32 = jnp.uint32
QUAD = ((0, 0), (0, 1), (1, 0), (1, 1))


class _Blocks:
    def __init__(self, v):
        self.v = list(v)

    def __add__(self, o):
        return _Blocks(a + b for a, b in zip(self.v, o.v))

    def __sub__(self, o):
        return _Blocks(a - b for a, b in zip(self.v, o.v))


def _rhs_sums(B11, B12, B21, B22):
    yield B11 - B22
    yield B11
    yield B12 + B22
    yield B21 + B11
    yield B22
    yield B11 + B12
    yield B21 + B22


def _strassen(A, mul, done):
    A11, A12, A21, A22 = A
    M2 = mul(1, A21 - A22)
    M4 = mul(3, A22)
    done(2, M2 + M4)
    M3 = mul(2, A11)
    M5 = mul(4, A12 - A11)
    done(1, M3 + M5)
    M1 = mul(0, A11 - A22)
    done(3, ((M3 - M2) + M1) + mul(5, A21 - A11))
    done(0, ((M4 - M5) + M1) + mul(6, A12 - A22))


SWAP = (0, 1, 0, 0, 1, 1, 1)


def _kernel(x0_ref, ws_hbm, bs_ref, o_ref, w_ref, wc_ref, bb_ref, x_ref, sems, *, head):
    L, D, _ = w_ref.shape
    d = D // 4

    def col(J, j, swap, off=0, size=d):
        start = (2 * (J ^ swap) + j) * d + off
        return pl.ds(start if isinstance(start, int) else pl.multiple_of(start, 128), size)

    def tile_blocks(s, swap):
        return [[(pl.ds((4 * s + 2 * I + i) * H2, H2), col(J, j, swap)) for i, j in QUAD] for I, J in QUAD]

    def load(ref, s, swap=0):
        return [_Blocks(ref[b].astype(f32) for b in bq) for bq in tile_blocks(s, swap)]

    def store(ref, s, X, swap=0):
        for bq, Xq in zip(tile_blocks(s, swap), X):
            for b, v in zip(bq, Xq.v):
                ref[b] = v.astype(ref.dtype)

    def cross_layer(l, odd, X, X0s, Xs):
        def outer_mul(p, A):
            def mul(p2, a):
                w = jnp.concatenate([wc_ref.bitcast(u32)[l, 7 * p + p2, c] for c in range(d // 128)], axis=1)
                m = jnp.dot(a.astype(bf16), pltpu.bitcast(w, bf16), preferred_element_type=f32)
                if p in (2, 3) and p2 in (2, 3):
                    m = m + jnp.tile(bb_ref[l, :, col(3 - p, (3 - p2) ^ SWAP[p], odd)], (H2 // 8, 1))
                return m
            C = [None] * 4
            _strassen(A.v, mul, lambda q, c: C.__setitem__(q ^ SWAP[p], c))
            return _Blocks(C)

        Xn = [None] * 4

        def cross(q, proj):
            Xn[q] = _Blocks(x0 * c + x for x0, c, x in zip(X0s[q].v, proj.v, Xs[q].v))

        _strassen(X, outer_mul, cross)
        return Xn

    def weight_sums(l, odd, r, c):
        W = [_Blocks(w_ref[l, pl.ds((2 * I + i) * d + r, 16), col(J, j, odd, c * 128, 128)].astype(f32)
                     for i, j in QUAD) for I, J in QUAD]
        for p, Wp in enumerate(_rhs_sums(*W)):
            for p2, w in enumerate(_rhs_sums(*[Wp.v[q ^ SWAP[p]] for q in range(4)])):
                wc_ref[l, 7 * p + p2, c, pl.ds(r, 16), :] = w.astype(bf16)

    @pl.when(pl.program_id(0) == 0)
    def _first_step():
        copy = lambda l: pltpu.make_async_copy(ws_hbm.at[l], w_ref.at[l], sems.at[l])
        for l in range(AHEAD):
            copy(l).start()
        for l in range(L):
            bb_ref[l] = jnp.broadcast_to(bs_ref[l:l + 1, :].astype(f32), (8, D))
        x_ref[...] = x0_ref[:head, :].astype(f32)

        def prepare(l, odd):
            copy(l).wait()
            pl.when(l + AHEAD < L)(lambda: copy(l + AHEAD).start())
            for c in range(d // 128):
                pl.loop(0, d // 16)(lambda t: weight_sums(l, odd, pl.multiple_of(t * 16, 16), c))

        @pl.loop(0, L // 2)
        def _(h):
            for odd in range(2):
                l = 2 * h + odd
                prepare(l, odd)
                for s in range(head // (4 * H2)):
                    Xn = cross_layer(l, odd, load(x_ref, s), load(x0_ref, s, odd), load(x_ref, s, odd))
                    store(x_ref, s, Xn, odd)

        o_ref[:head, :] = x_ref[...].astype(o_ref.dtype)

    @pl.when(pl.program_id(0) > 0)
    def _steady_step():
        for s in range(NS):
            X0 = X = load(x0_ref, s)
            for l in range(L):
                swap = lambda Y: [Y[q ^ (l % 2)] for q in range(4)]
                X = swap(cross_layer(l, l % 2, X, swap(X0), swap(X)))
            store(o_ref, s, X)


@jax.jit
def pallas_standalone__cross_network_dcn__recsys_kernel(x0, ws, bs):
    B, D = x0.shape
    L = ws.shape[0]
    d = D // 4
    TM = 4 * H2 * NS
    steps = pl.cdiv(B, TM)
    head = B - (steps - 1) * TM
    rows = lambda i: (jnp.where(i == 0, steps - 1, i - 1), 0)
    return pl.pallas_call(
        functools.partial(_kernel, head=head),
        grid=(steps,),
        in_specs=[
            pl.BlockSpec((TM, D), rows),
            pl.BlockSpec(memory_space=pl.ANY),
            pl.BlockSpec((L, D), lambda i: (0, 0)),
        ],
        out_specs=pl.BlockSpec((TM, D), rows),
        out_shape=jax.ShapeDtypeStruct((B, D), x0.dtype),
        scratch_shapes=[
            pltpu.VMEM((L, D, D), ws.dtype),
            pltpu.VMEM((L, 49, d // 128, d, 128), bf16),
            pltpu.VMEM((L, 8, D), f32),
            pltpu.VMEM((head, D), f32),
            pltpu.SemaphoreType.DMA((L,)),
        ],
        compiler_params=pltpu.CompilerParams(
            dimension_semantics=("arbitrary",), vmem_limit_bytes=100 * 1024 * 1024, flags=FLAGS),
    )(x0, ws, bs)
```

```python
import jax
import jax.numpy as jnp
import jax.experimental.pallas as pl
import jax.experimental.pallas.tpu as pltpu

H = 64
NS = 2
FLAGS = {"XLA_TPU_FORCE_LP_LLO_SCHEDULER": True}
f32 = jnp.float32
bf16 = jnp.bfloat16
QUAD = ((0, 0), (0, 1), (1, 0), (1, 1))

MAX_SUMSQ_PRODUCT = 0.32
UNDERFLOW = 1e-33

SWAP = (0, 1, 0, 0, 1, 1, 1)


class _Blocks:
    def __init__(self, v):
        self.v = list(v)

    def __add__(self, o):
        return _Blocks(a + b for a, b in zip(self.v, o.v))

    def __sub__(self, o):
        return _Blocks(a - b for a, b in zip(self.v, o.v))

    def sumsq(self):
        a, b, c, d = [v * v for v in self.v]
        return ((c + b) + d) + a


def _rhs_sums(B11, B12, B21, B22):
    yield B11 - B22
    yield B11
    yield B12 + B22
    yield B21 + B11
    yield B22
    yield B11 + B12
    yield B21 + B22


def _strassen(A, mul, done):
    A11, A12, A21, A22 = A
    M2 = mul(1, A21 - A22)
    M4 = mul(3, A22)
    done(2, M2 + M4)
    M3 = mul(2, A11)
    M5 = mul(4, A12 - A11)
    done(1, M3 + M5)
    M1 = mul(0, A11 - A22)
    done(3, ((M3 - M2) + M1) + mul(5, A21 - A11))
    done(0, ((M4 - M5) + M1) + mul(6, A12 - A22))


def _kernel(x0_ref, ws_hbm, bs_ref, o_ref, w_ref, wc_ref, bb_ref, lim_ref, x_ref, plain_ref, sems):
    L, D, _ = w_ref.shape
    d = D // 4
    step = pl.program_id(0)

    def col(J, j, swap, off=0, size=d):
        return pl.ds((2 * (J ^ swap) + j) * d + off, size)

    def tile_blocks(s, swap):
        return [[(pl.ds((4 * s + 2 * I + i) * H, H), col(J, j, swap)) for i, j in QUAD] for I, J in QUAD]

    def load(ref, s, swap=0):
        return [_Blocks(ref[b].astype(f32) for b in bq) for bq in tile_blocks(s, swap)]

    def store(ref, s, X, swap=0):
        for bq, Xq in zip(tile_blocks(s, swap), X):
            for b, v in zip(bq, Xq.v):
                ref[b] = v.astype(ref.dtype)

    def prepare_weights(l, odd):
        lim = None
        for c in range(d // 128):
            def rows(t, sumsq):
                r = pl.multiple_of(t * 16, 16)
                W = [_Blocks(w_ref[l, pl.ds((2 * I + i) * d + r, 16), col(J, j, odd, c * 128, 128)].astype(f32)
                             for i, j in QUAD) for I, J in QUAD]
                for p, Wp in enumerate(_rhs_sums(*W)):
                    for p2, w in enumerate(_rhs_sums(*[Wp.v[q ^ SWAP[p]] for q in range(4)])):
                        wc_ref[l, 7 * p + p2, c, pl.ds(r, 16), :] = w.astype(bf16)
                for Wq in W:
                    sumsq = sumsq + Wq.sumsq()
                return sumsq

            U = jax.lax.fori_loop(0, d // 16, rows, jnp.zeros((16, 128), f32))
            U = jnp.sum(U, axis=0, keepdims=True) + UNDERFLOW
            lim_c = jnp.where(U < jnp.inf, MAX_SUMSQ_PRODUCT / U - UNDERFLOW, -1.0)
            lim = lim_c if lim is None else jnp.minimum(lim, lim_c)
        lim_ref[l] = jnp.broadcast_to(jnp.min(lim, axis=1, keepdims=True), (8, 128))

    def check(l, X, unsafe):
        T = None
        for q in (2, 1, 3, 0):
            s = X[q].sumsq()
            for c in range(0, d, 128):
                T = s[:, c:c + 128] if T is None else T + s[:, c:c + 128]
        T = jnp.sum(T, axis=1, keepdims=True)
        return jnp.where(T <= jnp.tile(lim_ref[l], (H // 8, 1)), unsafe, 1.0)

    def cross_layer(l, odd, X, X0s, Xs):
        def outer_mul(p, A):
            def mul(p2, a):
                w = jnp.concatenate(
                    [wc_ref.bitcast(jnp.uint32)[l, 7 * p + p2, c] for c in range(d // 128)], axis=1)
                m = jnp.dot(a.astype(bf16), pltpu.bitcast(w, bf16), preferred_element_type=f32)
                if p in (2, 3) and p2 in (2, 3):
                    m = m + jnp.tile(bb_ref[l, :, col(3 - p, (3 - p2) ^ SWAP[p], odd)], (H // 8, 1))
                return m
            C = [None] * 4
            _strassen(A.v, mul, lambda q, c: C.__setitem__(q ^ SWAP[p], c))
            return _Blocks(C)

        Xn = [None] * 4

        def cross(q, proj):
            Xn[q] = _Blocks(x0 * c + x for x0, c, x in zip(X0s[q].v, proj.v, Xs[q].v))

        _strassen(X, outer_mul, cross)
        return Xn

    def report(unsafe):
        plain_ref[0] = (jnp.max(unsafe) > 0.0).astype(jnp.int32)

    @pl.when(step == 0)
    def _first_step():
        copy = lambda l: pltpu.make_async_copy(ws_hbm.at[l], w_ref.at[l], sems.at[l])
        for l in range(L):
            copy(l).start()
        for l in range(L):
            bb_ref[l] = jnp.broadcast_to(bs_ref[l:l + 1, :].astype(f32), (8, D))
        x_ref[...] = x0_ref[...].astype(f32)

        def layer(l, odd, unsafe):
            copy(l).wait()
            prepare_weights(l, odd)
            for s in range(NS):
                X = load(x_ref, s)
                unsafe = check(l, X, unsafe)
                store(x_ref, s, cross_layer(l, odd, X, load(x0_ref, s, odd), load(x_ref, s, odd)), odd)
            return unsafe

        unsafe = jax.lax.fori_loop(
            0, L // 2, lambda h, u: layer(2 * h + 1, 1, layer(2 * h, 0, u)), jnp.zeros((H, 128), f32))
        if L % 2:
            unsafe = layer(L - 1, 0, unsafe)
        o_ref[...] = x_ref[...].astype(o_ref.dtype)
        report(unsafe)

    @pl.when(step > 0)
    def _later_step():
        @pl.when(plain_ref[0] == 0)
        def _():
            unsafe = jnp.zeros((H, 128), f32)
            for s in range(NS):
                X0 = X = load(x0_ref, s)
                for l in range(L):
                    swap = lambda Y: [Y[q ^ (l % 2)] for q in range(4)]
                    unsafe = check(l, X, unsafe)
                    X = swap(cross_layer(l, l % 2, X, swap(X0), swap(X)))
                store(o_ref, s, X)
            report(unsafe)

    @pl.when(plain_ref[0] != 0)
    def _plain_matmuls():
        x_ref[...] = x0_ref[...].astype(f32)

        @pl.loop(0, L)
        def _(l):
            x = x_ref[...]
            proj = jnp.dot(x.astype(bf16), w_ref[l], preferred_element_type=f32)
            bias = jnp.tile(bb_ref[l], (x.shape[0] // 8, 1))
            x_ref[...] = x0_ref[...].astype(f32) * (proj + bias) + x

        o_ref[...] = x_ref[...].astype(o_ref.dtype)


@jax.jit
def pallas_standalone__cross_network_dcn__recsys_kernel(x0, ws, bs):
    B, D = x0.shape
    L = ws.shape[0]
    d = D // 4
    TM = 4 * H * NS
    assert B % TM == 0 and d % 128 == 0 and ws.dtype == bf16
    return pl.pallas_call(
        _kernel,
        grid=(B // TM,),
        in_specs=[
            pl.BlockSpec((TM, D), lambda i: (i, 0)),
            pl.BlockSpec(memory_space=pl.ANY),
            pl.BlockSpec((L, D), lambda i: (0, 0)),
        ],
        out_specs=pl.BlockSpec((TM, D), lambda i: (i, 0)),
        out_shape=jax.ShapeDtypeStruct((B, D), x0.dtype),
        scratch_shapes=[
            pltpu.VMEM((L, D, D), bf16),
            pltpu.VMEM((L, 49, d // 128, d, 128), bf16),
            pltpu.VMEM((L, 8, D), f32),
            pltpu.VMEM((L, 8, 128), f32),
            pltpu.VMEM((TM, D), f32),
            pltpu.SMEM((1,), jnp.int32),
            pltpu.SemaphoreType.DMA((L,)),
        ],
        compiler_params=pltpu.CompilerParams(
            dimension_semantics=("arbitrary",), vmem_limit_bytes=100 * 1024 * 1024, flags=FLAGS),
    )(x0, ws, bs)
```

```python
import jax
import jax.numpy as jnp
import jax.experimental.pallas as pl
import jax.experimental.pallas.tpu as pltpu

TM = 512
f32 = jnp.float32


def _kernel(x0_ref, ws_hbm, bs_ref, o_ref, w_ref, b_ref, x_ref, sems):
    L, D, _ = w_ref.shape

    def cross_layer(l, x0, x):
        proj = jnp.dot(x.astype(w_ref.dtype), w_ref[l], preferred_element_type=f32)
        return x0 * (proj + jnp.tile(b_ref[l], (TM // 8, 1))) + x

    @pl.when(pl.program_id(0) == 0)
    def _first_step():
        copy = lambda l: pltpu.make_async_copy(ws_hbm.at[l], w_ref.at[l], sems.at[l])
        for l in range(L):
            copy(l).start()
        for l in range(L):
            b_ref[l] = jnp.broadcast_to(bs_ref[l:l + 1, :].astype(f32), (8, D))
        x_ref[...] = x0_ref[...].astype(f32)

        @pl.loop(0, L)
        def _(l):
            copy(l).wait()
            x_ref[...] = cross_layer(l, x0_ref[...].astype(f32), x_ref[...])

        o_ref[...] = x_ref[...].astype(o_ref.dtype)

    @pl.when(pl.program_id(0) > 0)
    def _later_step():
        x = x0 = x0_ref[...].astype(f32)
        for l in range(L):
            x = cross_layer(l, x0, x)
        o_ref[...] = x.astype(o_ref.dtype)


@jax.jit
def pallas_standalone__cross_network_dcn__recsys_kernel(x0, ws, bs):
    B, D = x0.shape
    L = ws.shape[0]
    assert B % TM == 0
    return pl.pallas_call(
        _kernel,
        grid=(B // TM,),
        in_specs=[
            pl.BlockSpec((TM, D), lambda i: (i, 0)),
            pl.BlockSpec(memory_space=pl.ANY),
            pl.BlockSpec((L, D), lambda i: (0, 0)),
        ],
        out_specs=pl.BlockSpec((TM, D), lambda i: (i, 0)),
        out_shape=jax.ShapeDtypeStruct((B, D), x0.dtype),
        scratch_shapes=[
            pltpu.VMEM((L, D, D), ws.dtype),
            pltpu.VMEM((L, 8, D), f32),
            pltpu.VMEM((TM, D), f32),
            pltpu.SemaphoreType.DMA((L,)),
        ],
        compiler_params=pltpu.CompilerParams(
            dimension_semantics=("arbitrary",), vmem_limit_bytes=64 * 1024 * 1024),
    )(x0, ws, bs)
```

```python
import jax
import jax.numpy as jnp
import jax.experimental.pallas as pl
import jax.experimental.pallas.tpu as pltpu

TM = 512
PARTS = 4
f32 = jnp.float32


def _kernel(x0_ref, ws_hbm, bs_ref, o_ref, w_ref, b_ref, x_ref, sems):
    L, D, _ = w_ref.shape
    n = D // PARTS

    def cross(x0, x, lhs, w, b):
        proj = jnp.dot(lhs, w, preferred_element_type=f32)
        return x0 * (proj + jnp.tile(b, (x.shape[0] // 8, 1))) + x

    @pl.when(pl.program_id(0) == 0)
    def _first_step():
        def part_copy(c, cols):
            return pltpu.make_async_copy(ws_hbm.at[0, :, cols], w_ref.at[0, :, cols], sems.at[L - 1 + c])

        def layer_copy(l):
            return pltpu.make_async_copy(ws_hbm.at[l], w_ref.at[l], sems.at[l - 1])

        for c in range(PARTS):
            part_copy(c, pl.ds(c * n, n)).start()
        for l in range(1, L):
            layer_copy(l).start()
        for l in range(L):
            b_ref[l] = jnp.broadcast_to(bs_ref[l:l + 1, :].astype(f32), (8, D))

        @pl.loop(0, PARTS)
        def _(c):
            cols = pl.ds(pl.multiple_of(c * n, n), n)
            part_copy(c, cols).wait()
            x0 = x0_ref[:, cols].astype(f32)
            x_ref[:, cols] = cross(x0, x0, x0_ref[...], w_ref[0, :, cols], b_ref[0, :, cols])

        @pl.loop(1, L)
        def _(l):
            layer_copy(l).wait()
            x = x_ref[...]
            x_ref[...] = cross(x0_ref[...].astype(f32), x, x.astype(w_ref.dtype), w_ref[l], b_ref[l])

        o_ref[...] = x_ref[...].astype(o_ref.dtype)

    @pl.when(pl.program_id(0) > 0)
    def _later_step():
        x = x0 = x0_ref[...].astype(f32)
        for l in range(L):
            x = cross(x0, x, x.astype(w_ref.dtype), w_ref[l], b_ref[l])
        o_ref[...] = x.astype(o_ref.dtype)


@jax.jit
def pallas_standalone__cross_network_dcn__recsys_kernel(x0, ws, bs):
    B, D = x0.shape
    L = ws.shape[0]
    assert B % TM == 0 and D % (128 * PARTS) == 0 and x0.dtype == ws.dtype
    return pl.pallas_call(
        _kernel,
        grid=(B // TM,),
        in_specs=[
            pl.BlockSpec((TM, D), lambda i: (i, 0)),
            pl.BlockSpec(memory_space=pl.ANY),
            pl.BlockSpec((L, D), lambda i: (0, 0)),
        ],
        out_specs=pl.BlockSpec((TM, D), lambda i: (i, 0)),
        out_shape=jax.ShapeDtypeStruct((B, D), x0.dtype),
        scratch_shapes=[
            pltpu.VMEM((L, D, D), ws.dtype),
            pltpu.VMEM((L, 8, D), f32),
            pltpu.VMEM((TM, D), f32),
            pltpu.SemaphoreType.DMA((L - 1 + PARTS,)),
        ],
        compiler_params=pltpu.CompilerParams(
            dimension_semantics=("arbitrary",), vmem_limit_bytes=64 * 1024 * 1024),
    )(x0, ws, bs)
```
